```python
import os as _os
_os.environ.setdefault("JAX_PLATFORMS", "cpu")
import jax
import jax.numpy as jnp

def _softmax(x, axis=-1):
    return jax.nn.softmax(x, axis=axis)
def _gelu(x):
    return jax.nn.gelu(x, approximate=True)
def _silu(x):
    return jax.nn.silu(x)
def _sigmoid(x):
    return jax.nn.sigmoid(x)
def _layernorm(x, axis=-1, eps=1e-5):
    m = jnp.mean(x, axis=axis, keepdims=True)
    v = jnp.var(x, axis=axis, keepdims=True)
    return (x - m) / jnp.sqrt(v + eps)
def _scatter_add(tgt, idx, src, axis=0):
    return tgt.at[idx].add(src)
def _segment_sum(src, seg, n):
    return jax.ops.segment_sum(src, seg, n)
class _Rng:
    def __init__(self, key):
        self._k = key
    def _next(self):
        self._k, sub = jax.random.split(self._k)
        return sub
    def normal(self, shape):
        return jax.random.normal(self._next(), shape, dtype=jnp.bfloat16)
    def randint(self, lo, hi, shape):
        return jax.random.randint(self._next(), shape, lo, hi, dtype=jnp.int32)
    def uniform(self, shape, lo=0.0, hi=1.0):
        return jax.random.uniform(self._next(), shape, jnp.bfloat16, lo, hi)
    def permutation(self, n):
        return jax.random.permutation(self._next(), n)


kernel_name = 'recurrent_scan__ssm_conv_s5__mixer_s_mlp__prompt'

def setup_inputs():
    _rng = _Rng(jax.random.key(int.from_bytes(__import__("os").urandom(4), "little")))
    _w = (lambda a: (lambda t: t.astype(jnp.bfloat16) if jnp.issubdtype(t.dtype, jnp.floating) else t)(jnp.asarray(a)))
    def _A_setup():
        B, S, D = 1, 2048, 640
        P = D
        Lambda_re = -0.5 * jnp.exp((lambda *s: _rng.normal(s) * 0.8)(P))
        Lambda_im = (lambda *s: _rng.normal(s) * 0.8)(P) * 1.0
        B_re = (lambda *s: _rng.normal(s) * 0.8)(P, D) * (D ** -0.5)
        B_im = (lambda *s: _rng.normal(s) * 0.8)(P, D) * (D ** -0.5)
        C_re = (lambda *s: _rng.normal(s) * 0.8)(D, P) * (P ** -0.5)
        C_im = (lambda *s: _rng.normal(s) * 0.8)(D, P) * (P ** -0.5)
        log_dt = (lambda *s: _rng.normal(s) * 0.8)(P) * 0.3 - 2.0
        Dskip = (lambda *s: _rng.normal(s) * 0.8)(D)
        return {
            "x": _w((lambda *s: _rng.normal(s) * 0.05)(B, S, D)),
            "Lambda_re": _w(Lambda_re),
            "Lambda_im": _w(Lambda_im),
            "B_re": _w(B_re),
            "B_im": _w(B_im),
            "C_re": _w(C_re),
            "C_im": _w(C_im),
            "log_dt": _w(log_dt),
            "Dskip": _w(Dskip),
        }
    _A_in = _A_setup()

    def _B_setup():
        B, S, D, F = 1, 2048, 640, 1536
        return {
            "x":  _w((lambda *s: _rng.normal(s) * 0.05)(B, S, D)),
            "w1": _w((lambda *s: _rng.normal(s) * 0.8)(D, D) * (D ** -0.5)),
            "w2": _w((lambda *s: _rng.normal(s) * 0.8)(D, D) * (D ** -0.5)),
            "w3": _w((lambda *s: _rng.normal(s) * 0.8)(D, F) * (D ** -0.5)),
            "w4": _w((lambda *s: _rng.normal(s) * 0.8)(F, D) * (F ** -0.5)),
        }
    _B_in = _B_setup()

    return {
        "A_x": _A_in["x"],
        "A_Lambda_re": _A_in["Lambda_re"],
        "A_Lambda_im": _A_in["Lambda_im"],
        "A_B_re": _A_in["B_re"],
        "A_B_im": _A_in["B_im"],
        "A_C_re": _A_in["C_re"],
        "A_C_im": _A_in["C_im"],
        "A_log_dt": _A_in["log_dt"],
        "A_Dskip": _A_in["Dskip"],
        "B_x": _B_in["x"],
        "B_w1": _B_in["w1"],
        "B_w2": _B_in["w2"],
        "B_w3": _B_in["w3"],
        "B_w4": _B_in["w4"],
    }

def reference(A_x, A_Lambda_re, A_Lambda_im, A_B_re, A_B_im, A_C_re, A_C_im, A_log_dt, A_Dskip, B_x, B_w1, B_w2, B_w3, B_w4):
    def _A_ref(x, Lambda_re, Lambda_im, B_re, B_im, C_re, C_im, log_dt, Dskip):
        Bsz, L, H = x.shape
        Lam = Lambda_re + 1j * Lambda_im
        Bmat = B_re + 1j * B_im
        Cmat = C_re + 1j * C_im
        dt = jnp.exp(log_dt)
        Lam_bar = jnp.exp(dt * Lam)
        B_bar = ((Lam_bar - 1.0) / Lam)[:, None] * Bmat
        Bu = jnp.einsum("bld,pd->blp", x + 0j, B_bar)
        h = jnp.zeros_like(Bu[:, 0, :])
        hs = []
        for t in range(L):
            h = Lam_bar[None, :] * h + Bu[:, t, :]
            hs.append(h)
        hseq = jnp.stack(hs, 1)
        y = 2.0 * jnp.einsum("blp,dp->bld", hseq, Cmat).real + x * Dskip[None, None, :]
        return y

    def _B_ref(x, w1, w2, w3, w4):
        B, S, D = x.shape
        h = _gelu(_layernorm(x, axis=-1) @ w1)
        c = D // 4
        g0 = jnp.pad(h[:, :, 0*c:1*c], ((0, 0), (1, 0), (0, 0)))[:, :S, :]
        g1 = jnp.pad(h[:, :, 1*c:2*c], ((0, 0), (0, 1), (0, 0)))[:, 1:, :]
        g2 = jnp.pad(h[:, :, 2*c:3*c], ((0, 0), (2, 0), (0, 0)))[:, :S, :]
        g3 = jnp.pad(h[:, :, 3*c:   ], ((0, 0), (0, 2), (0, 0)))[:, 2:, :]
        hs = jnp.concatenate([g0, g1, g2, g3], axis=-1) @ w2
        x1 = x + hs
        h2 = _gelu(_layernorm(x1, axis=-1) @ w3) @ w4
        return x1 + h2

    x = A_x
    xn = _layernorm(x, axis=-1)
    s = _A_ref(xn, A_Lambda_re, A_Lambda_im, A_B_re, A_B_im, A_C_re, A_C_im, A_log_dt, A_Dskip)
    g = _silu(_B_ref(xn, B_w1, B_w2, B_w3, B_w4))
    return x + s * g
```

```python
import functools

import jax
import jax.numpy as jnp
from jax import lax
import jax.experimental.pallas as pl
import jax.experimental.pallas.tpu as pltpu

_EPS = 1e-5
_T = 256
_NC = 8
_CS = _T // _NC
_HALO = 16


def _ln(x):
    m = jnp.mean(x, axis=-1, keepdims=True)
    xc = x - m
    v = jnp.mean(xc * xc, axis=-1, keepdims=True)
    return xc * lax.rsqrt(v + _EPS)


def _gelu(x):
    c = 0.7978845608028654
    return 0.5 * x * (1.0 + jnp.tanh(c * (x + 0.044715 * (x * x * x))))


def _dot_nn(a, b):
    return jnp.dot(a, b, preferred_element_type=jnp.float32)


def _dot_nt(a, b):
    return lax.dot_general(a, b, (((1,), (1,)), ((), ())),
                           preferred_element_type=jnp.float32)


def _cmul(ar, ai, br, bi):
    return ar * br - ai * bi, ar * bi + ai * br


def _kernel(x_ref, lre_ref, lim_ref, bre_ref, bim_ref, cre_ref, cim_ref,
            ldt_ref, dsk_ref, w1_ref, w2_ref, w3_ref, w4_ref, o_ref,
            par_ref, carry_ref, ure_ref, uim_ref, h1_ref, *, L, D):
    T, CS = _T, _CS
    i = pl.program_id(0)
    nsteps = pl.num_programs(0)
    f32 = jnp.float32
    bf16 = jnp.bfloat16

    @pl.when(i == 0)
    def _():
        lre = lre_ref[...].astype(f32)
        lim = lim_ref[...].astype(f32)
        dt = jnp.exp(ldt_ref[...].astype(f32)).astype(bf16).astype(f32)
        mag = jnp.exp(dt * lre)
        ang = dt * lim
        ar = mag * jnp.cos(ang)
        ai = mag * jnp.sin(ang)
        den = lre * lre + lim * lim
        nr = ar - 1.0
        ni = ai
        cr = (nr * lre + ni * lim) / den
        ci = (ni * lre - nr * lim) / den
        par_ref[0:1, :] = ar
        par_ref[1:2, :] = ai
        par_ref[2:3, :] = cr
        par_ref[3:4, :] = ci
        pr, pi = ar, ai
        n = 1
        while n < CS:
            pr, pi = _cmul(pr, pi, pr, pi)
            n *= 2
        for k in range(3):
            par_ref[4 + 2 * k:5 + 2 * k, :] = pr
            par_ref[5 + 2 * k:6 + 2 * k, :] = pi
            pr, pi = _cmul(pr, pi, pr, pi)
        carry_ref[...] = jnp.zeros(carry_ref.shape, f32)
        h1_ref[0:8, :] = jnp.zeros((8, D), f32)

    row0 = pl.multiple_of(i * T, T)
    xm = x_ref[pl.ds(row0, T), :].astype(f32)
    halo0 = pl.multiple_of(jnp.minimum(row0 + T, L - _HALO), _HALO)
    xa = x_ref[pl.ds(halo0, _HALO), :].astype(f32)
    xall = jnp.concatenate([xm, xa], axis=0)
    xn_all = _ln(xall).astype(bf16)
    xn_b = xn_all[:T]
    xn = xn_b.astype(f32)

    ur = _dot_nt(xn_b, bre_ref[...])
    ui = _dot_nt(xn_b, bim_ref[...])
    cr = par_ref[2:3, :]
    ci = par_ref[3:4, :]
    bur, bui = _cmul(cr, ci, ur, ui)
    NJ = D // 128
    for j in range(NJ):
        ure_ref[j] = bur[:, 128 * j:128 * (j + 1)]
        uim_ref[j] = bui[:, 128 * j:128 * (j + 1)]

    xnn = _ln(xn_all.astype(f32)).astype(bf16)
    h1 = _gelu(_dot_nn(xnn, w1_ref[...]))
    h1_ref[8:8 + T, :] = h1[:T]
    is_last = i == nsteps - 1
    h1_ref[8 + T:8 + T + _HALO, :] = jnp.where(is_last, 0.0, h1[T:])

    def ld(ref, s):
        return jnp.concatenate(
            [ref[j, pl.ds(s, _NC, stride=CS), :] for j in range(NJ)], axis=1)

    def st(ref, s, v):
        for j in range(NJ):
            ref[j, pl.ds(s, _NC, stride=CS), :] = v[:, 128 * j:128 * (j + 1)]

    ar = jnp.broadcast_to(par_ref[0:1, :], (_NC, D))
    ai = jnp.broadcast_to(par_ref[1:2, :], (_NC, D))
    er = jnp.zeros((_NC, D), f32)
    ei = jnp.zeros((_NC, D), f32)
    for s in range(CS):
        br = ld(ure_ref, s)
        bi = ld(uim_ref, s)
        er, ei = ar * er - ai * ei + br, ar * ei + ai * er + bi
    sub = lax.broadcasted_iota(jnp.int32, (_NC, D), 0)
    zr = jnp.where(sub == 0, pltpu.roll(carry_ref[0], 1, 0), pltpu.roll(er, 1, 0))
    zi = jnp.where(sub == 0, pltpu.roll(carry_ref[1], 1, 0), pltpu.roll(ei, 1, 0))
    for k in range(3):
        sh = 1 << k
        pr = par_ref[4 + 2 * k:5 + 2 * k, :]
        pi = par_ref[5 + 2 * k:6 + 2 * k, :]
        sr = jnp.where(sub >= sh, pltpu.roll(zr, sh, 0), 0.0)
        si = jnp.where(sub >= sh, pltpu.roll(zi, sh, 0), 0.0)
        tr, ti = _cmul(pr, pi, sr, si)
        zr = zr + tr
        zi = zi + ti
    hr, hi = zr, zi
    for s in range(CS):
        br = ld(ure_ref, s)
        bi = ld(uim_ref, s)
        hr, hi = ar * hr - ai * hi + br, ar * hi + ai * hr + bi
        st(ure_ref, s, hr)
        st(uim_ref, s, hi)
    carry_ref[0] = hr
    carry_ref[1] = hi

    hre_b = jnp.concatenate([ure_ref[j] for j in range(NJ)], axis=1).astype(bf16)
    him_b = jnp.concatenate([uim_ref[j] for j in range(NJ)], axis=1).astype(bf16)
    y = _dot_nt(hre_b, cre_ref[...]) - _dot_nt(him_b, cim_ref[...])
    y = 2.0 * y + xn * dsk_ref[...].astype(f32)

    lane = lax.broadcasted_iota(jnp.int32, (T, 128), 1)
    s0 = h1_ref[7:7 + T, 0:128]
    s1 = jnp.where(lane < 32, h1_ref[7:7 + T, 128:256], h1_ref[9:9 + T, 128:256])
    s2 = jnp.where(lane < 64, h1_ref[9:9 + T, 256:384], h1_ref[6:6 + T, 256:384])
    s3 = jnp.where(lane < 96, h1_ref[6:6 + T, 384:512], h1_ref[10:10 + T, 384:512])
    s4 = h1_ref[10:10 + T, 512:640]
    sh_all = jnp.concatenate([s0, s1, s2, s3, s4], axis=1).astype(bf16)
    h1_ref[0:8, :] = h1_ref[T:T + 8, :]
    x1 = xn + _dot_nn(sh_all, w2_ref[...])
    h2 = _gelu(_dot_nn(_ln(x1).astype(bf16), w3_ref[...])).astype(bf16)
    z = x1 + _dot_nn(h2, w4_ref[...])
    g = z * (1.0 / (1.0 + jnp.exp(-z)))
    o_ref[...] = xm + y * g


@jax.jit
def pallas_recurrent_scan__ssm_conv_s5__mixer_s_mlp__prompt_kernel(
    A_x: jax.Array,
    A_Lambda_re: jax.Array,
    A_Lambda_im: jax.Array,
    A_B_re: jax.Array,
    A_B_im: jax.Array,
    A_C_re: jax.Array,
    A_C_im: jax.Array,
    A_log_dt: jax.Array,
    A_Dskip: jax.Array,
    B_x: jax.Array,
    B_w1: jax.Array,
    B_w2: jax.Array,
    B_w3: jax.Array,
    B_w4: jax.Array,
):
    Bsz, L, D = A_x.shape
    P = A_Lambda_re.shape[0]
    F = B_w3.shape[1]
    assert Bsz == 1 and D == 640 and P == 640 and L % _T == 0
    x2 = A_x.reshape(L, D)
    row = lambda v: v.reshape(1, -1)

    full = lambda shape: pl.BlockSpec(shape, lambda i: (0,) * len(shape))
    out = pl.pallas_call(
        functools.partial(_kernel, L=L, D=D),
        grid=(L // _T,),
        in_specs=[
            full((L, D)),
            full((1, P)), full((1, P)),
            full((P, D)), full((P, D)),
            full((D, P)), full((D, P)),
            full((1, P)), full((1, D)),
            full((D, D)), full((D, D)), full((D, F)), full((F, D)),
        ],
        out_specs=pl.BlockSpec((_T, D), lambda i: (i, 0)),
        out_shape=jax.ShapeDtypeStruct((L, D), jnp.float32),
        scratch_shapes=[
            pltpu.VMEM((16, P), jnp.float32),
            pltpu.VMEM((2, _NC, P), jnp.float32),
            pltpu.VMEM((P // 128, _T, 128), jnp.float32),
            pltpu.VMEM((P // 128, _T, 128), jnp.float32),
            pltpu.VMEM((_T + 8 + _HALO, D), jnp.float32),
        ],
        compiler_params=pltpu.CompilerParams(
            dimension_semantics=("arbitrary",),
            vmem_limit_bytes=100 * 1024 * 1024,
        ),
    )(x2, row(A_Lambda_re), row(A_Lambda_im), A_B_re, A_B_im, A_C_re, A_C_im,
      row(A_log_dt), row(A_Dskip), B_w1, B_w2, B_w3, B_w4)
    return out.reshape(Bsz, L, D)
```

```python
import functools

import jax
import jax.numpy as jnp
from jax import lax
import jax.experimental.pallas as pl
import jax.experimental.pallas.tpu as pltpu

_EPS = 1e-5
_T = 256
_NV = 2
_NC = 8 * _NV
_CS = _T // _NC + 1
_TP = _CS * _NC
_HALO = 16
_RC = 32
_X0 = 2 * _T + _HALO
_X1 = 3 * _T + _HALO


def _ln(x):
    m = jnp.mean(x, axis=-1, keepdims=True)
    xc = x - m
    v = jnp.mean(xc * xc, axis=-1, keepdims=True)
    return xc * lax.rsqrt(v + _EPS)


def _gelu(x):
    c = 0.7978845608028654
    hx = 0.5 * x
    return hx + hx * jnp.tanh(x * (c + (c * 0.044715) * (x * x)))


def _dot_nn(a, b):
    return jnp.dot(a, b, preferred_element_type=jnp.float32)


def _dot_nt(a, b):
    return lax.dot_general(a, b, (((1,), (1,)), ((), ())),
                           preferred_element_type=jnp.float32)


def _cmul(ar, ai, br, bi):
    return ar * br - ai * bi, ar * bi + ai * br


def _kernel(x_hbm, lre_hbm, lim_hbm, ldt_hbm, dsk_hbm,
            bre_hbm, bim_hbm, cre_hbm, cim_hbm, w1_hbm, w2_hbm, w3_hbm, w4_hbm,
            o_ref,
            x_ref, lre_ref, lim_ref, ldt_ref, dsk_ref,
            bre_ref, bim_ref, cre_ref, cim_ref, w1_ref, w2_ref, w3_ref, w4_ref,
            sems, par_ref, carry_ref, *bufs, L, D):
    T, CS, NV = _T, _CS, _NV
    NJ = D // 128
    i = pl.program_id(0)
    nsteps = pl.num_programs(0)
    f32 = jnp.float32
    bf16 = jnp.bfloat16
    keys = ('ure', 'uim', 'h1', 'xn', 'xn2', 'xnn', 'hb')
    main = dict(zip(keys, bufs[:len(keys)]))
    alt = dict(zip(keys, bufs[len(keys):]))

    pairs = [
        ('vec0', lre_hbm, lre_ref), ('vec1', lim_hbm, lim_ref),
        ('vec2', ldt_hbm, ldt_ref), ('vec3', dsk_hbm, dsk_ref),
        ('x0', x_hbm.at[0:_T + _HALO], x_ref.at[0:_T + _HALO]),
        ('w1', w1_hbm, w1_ref),
        ('x0b', x_hbm.at[_T + _HALO:_X0], x_ref.at[_T + _HALO:_X0]), ('bre', bre_hbm, bre_ref), ('bim', bim_hbm, bim_ref),
        ('cre', cre_hbm, cre_ref), ('cim', cim_hbm, cim_ref), ('w2', w2_hbm, w2_ref),
        ('xa', x_hbm.at[_X0:_X1], x_ref.at[_X0:_X1]),
        ('w3', w3_hbm, w3_ref), ('w4', w4_hbm, w4_ref),
        ('x1', x_hbm.at[_X1:L], x_ref.at[_X1:L]),
    ]
    copies = {n: pltpu.make_async_copy(h, v, sems.at[k])
              for k, (n, h, v) in enumerate(pairs)}

    def wait(*ns):
        for n in ns:
            copies[n].wait()

    def init():
        lre = lre_ref[...].reshape(1, D).astype(f32)
        lim = lim_ref[...].reshape(1, D).astype(f32)
        dt = jnp.exp(ldt_ref[...].reshape(1, D).astype(f32)).astype(bf16).astype(f32)
        mag = jnp.exp(dt * lre)
        ang = dt * lim
        ar = mag * jnp.cos(ang)
        ai = mag * jnp.sin(ang)
        den = lre * lre + lim * lim
        nr = ar - 1.0
        ni = ai
        cr = (nr * lre + ni * lim) / den
        ci = (ni * lre - nr * lim) / den
        par_ref[0:1, :] = ar
        par_ref[1:2, :] = ai
        par_ref[2:3, :] = cr
        par_ref[3:4, :] = ci
        pr, pi = ar, ai
        n = 1
        while 2 * n <= CS:
            pr, pi = _cmul(pr, pi, pr, pi)
            n *= 2
        while n < CS:
            pr, pi = _cmul(pr, pi, ar, ai)
            n += 1
        for k in range(3):
            par_ref[4 + 2 * k:5 + 2 * k, :] = pr
            par_ref[5 + 2 * k:6 + 2 * k, :] = pi
            pr, pi = _cmul(pr, pi, pr, pi)
        par_ref[12:13, :] = dsk_ref[...].reshape(1, D).astype(f32)
        carry_ref[...] = jnp.zeros(carry_ref.shape, f32)
        for b in (main, alt):
            for j in range(NJ):
                b['ure'][j, T:_TP, :] = jnp.zeros((_TP - T, 128), f32)
                b['uim'][j, T:_TP, :] = jnp.zeros((_TP - T, 128), f32)

    def a_ln(blk, b):
        if isinstance(blk, int):
            row0 = blk * T
            hrow0 = row0 + T
        else:
            row0 = pl.multiple_of(blk * T, T)
            hrow0 = pl.multiple_of(jnp.minimum(row0 + T, L - _HALO), _HALO)

        def ln_rows(r0, nrows, src0):
            x = x_ref[pl.ds(src0, nrows), :].astype(f32)
            xn = _ln(x).astype(bf16)
            b['xn2'][r0:r0 + nrows, :] = xn
            b['xnn'][r0:r0 + nrows, :] = _ln(xn.astype(f32)).astype(bf16)

        for c in range(0, T, _RC):
            ln_rows(c, _RC, row0 + c)
        ln_rows(T, _HALO, hrow0)

    def a_store_u(b, ur, ui):
        bur, bui = _cmul(par_ref[2:3, :], par_ref[3:4, :], ur, ui)
        for j in range(NJ):
            b['ure'][j, 0:T, :] = bur[:, 128 * j:128 * (j + 1)]
            b['uim'][j, 0:T, :] = bui[:, 128 * j:128 * (j + 1)]

    def a_h1(b, prev, halo_zero):
        h1 = _gelu(_dot_nn(b['xnn'][...], w1_ref[...]))
        h1_ref = b['h1']
        if prev is None:
            h1_ref[0:8, :] = jnp.zeros((8, D), f32)
        else:
            h1_ref[0:8, :] = prev['h1'][T:T + 8, :]
        h1_ref[8:8 + T, :] = h1[:T]
        if halo_zero is None:
            h1_ref[8 + T:8 + T + _HALO, :] = h1[T:]
        else:
            h1_ref[8 + T:8 + T + _HALO, :] = jnp.where(halo_zero, 0.0, h1[T:])
        b['xn'][...] = b['xn2'][0:T, :]

    def a_scan(b):
        ure_ref, uim_ref = b['ure'], b['uim']
        ar = jnp.broadcast_to(par_ref[0:1, :], (8, D))
        ai = jnp.broadcast_to(par_ref[1:2, :], (8, D))
        sub = lax.broadcasted_iota(jnp.int32, (8, D), 0)

        def ld(ref, v, s):
            return jnp.concatenate(
                [ref[j, pl.ds(8 * CS * v + s, 8, stride=CS), :] for j in range(NJ)],
                axis=1)

        def st(ref, v, s, val):
            for j in range(NJ):
                ref[j, pl.ds(8 * CS * v + s, 8, stride=CS), :] = (
                    val[:, 128 * j:128 * (j + 1)])

        er = [jnp.zeros((8, D), f32) for _ in range(NV)]
        ei = [jnp.zeros((8, D), f32) for _ in range(NV)]
        for s in range(CS):
            for v in range(NV):
                br = ld(ure_ref, v, s)
                bi = ld(uim_ref, v, s)
                er[v], ei[v] = (ar * er[v] - ai * ei[v] + br,
                                ar * ei[v] + ai * er[v] + bi)
        inr, ini = carry_ref[0], carry_ref[1]
        hr, hi = [], []
        for v in range(NV):
            zr = jnp.where(sub == 0, pltpu.roll(inr, 1, 0), pltpu.roll(er[v], 1, 0))
            zi = jnp.where(sub == 0, pltpu.roll(ini, 1, 0), pltpu.roll(ei[v], 1, 0))
            for k in range(3):
                sh = 1 << k
                pr = par_ref[4 + 2 * k:5 + 2 * k, :]
                pi = par_ref[5 + 2 * k:6 + 2 * k, :]
                sr = jnp.where(sub >= sh, pltpu.roll(zr, sh, 0), 0.0)
                si = jnp.where(sub >= sh, pltpu.roll(zi, sh, 0), 0.0)
                tr, ti = _cmul(pr, pi, sr, si)
                zr = zr + tr
                zi = zi + ti
            hr.append(zr)
            hi.append(zi)
            if v + 1 < NV:
                tr, ti = _cmul(par_ref[4:5, :], par_ref[5:6, :], zr, zi)
                inr = tr + er[v]
                ini = ti + ei[v]
        for s in range(CS):
            for v in range(NV):
                br = ld(ure_ref, v, s)
                bi = ld(uim_ref, v, s)
                hr[v], hi[v] = (ar * hr[v] - ai * hi[v] + br,
                                ar * hi[v] + ai * hr[v] + bi)
                st(ure_ref, v, s, hr[v])
                st(uim_ref, v, s, hi[v])
        carry_ref[0] = jnp.concatenate(
            [ure_ref[j, T - 8:T, :] for j in range(NJ)], axis=1)
        carry_ref[1] = jnp.concatenate(
            [uim_ref[j, T - 8:T, :] for j in range(NJ)], axis=1)
        b['hb'][0] = jnp.concatenate([ure_ref[j, 0:T, :] for j in range(NJ)],
                                     axis=1).astype(bf16)
        b['hb'][1] = jnp.concatenate([uim_ref[j, 0:T, :] for j in range(NJ)],
                                     axis=1).astype(bf16)

    def stage_a(blk, halo_zero):
        xn_b = main['xn2'][0:T, :]
        ur = _dot_nt(xn_b, bre_ref[...])
        ui = _dot_nt(xn_b, bim_ref[...])
        a_store_u(main, ur, ui)
        a_h1(main, main, halo_zero)
        a_scan(main)

    def stage_b_early(b, first=False, c_late=False):
        lane = lax.broadcasted_iota(jnp.int32, (T, 128), 1)
        h1_ref = b['h1']
        xn = b['xn'][...].astype(f32)
        if not c_late:
            y = _dot_nt(b['hb'][0], cre_ref[...]) - _dot_nt(b['hb'][1], cim_ref[...])
            y = 2.0 * y + xn * par_ref[12:13, :]
        o = 8
        s0 = h1_ref[o - 1:o - 1 + T, 0:128]
        s1 = jnp.where(lane < 32, h1_ref[o - 1:o - 1 + T, 128:256],
                       h1_ref[o + 1:o + 1 + T, 128:256])
        s2 = jnp.where(lane < 64, h1_ref[o + 1:o + 1 + T, 256:384],
                       h1_ref[o - 2:o - 2 + T, 256:384])
        s3 = jnp.where(lane < 96, h1_ref[o - 2:o - 2 + T, 384:512],
                       h1_ref[o + 2:o + 2 + T, 384:512])
        s4 = h1_ref[o + 2:o + 2 + T, 512:640]
        sh_all = jnp.concatenate([s0, s1, s2, s3, s4], axis=1).astype(bf16)
        if first:
            wait('w2')
        x1 = xn + _dot_nn(sh_all, w2_ref[...])
        if c_late:
            never = i < 0
            h0 = jnp.where(never, x1.astype(bf16), b['hb'][0])
            y = _dot_nt(h0, cre_ref[...]) - _dot_nt(b['hb'][1], cim_ref[...])
            y = 2.0 * y + xn * par_ref[12:13, :]
        return x1, y

    def stage_b_late(x1, y, first=False, pin=False):
        row0 = pl.multiple_of(i * T, T)
        x1n = _ln(x1).astype(bf16)
        if first:
            wait('xa', 'w3')
            a_ln(2, main)
        if not pin:
            h2 = _gelu(_dot_nn(x1n, w3_ref[...])).astype(bf16)
        else:
            never = i < 0
            nt = w3_ref.shape[1] // 128
            parts = []
            for t in range(nt):
                p = _gelu(_dot_nn(x1n, w3_ref[:, 128 * t:128 * (t + 1)]))
                c = t - 2
                if 0 <= c <= T // _RC:
                    r0 = c * _RC
                    nr = _RC if c < T // _RC else _HALO
                    ja = main['xnn'][r0:r0 + nr, :].astype(f32)
                    jb = main['xn2'][r0:r0 + nr, :].astype(f32)
                    junk = jnp.concatenate(
                        [ja[:, 128 * j:128 * (j + 1)] + jb[:, 128 * j:128 * (j + 1)]
                         for j in range(NJ)] + [p[NJ * nr:]], axis=0)
                    p = jnp.where(never, junk, p)
                parts.append(p.astype(bf16))
            h2 = jnp.concatenate(parts, axis=1)
        if first:
            wait('w4')
        z = x1 + _dot_nn(h2, w4_ref[...])
        hz = 0.5 * z
        g = hz + hz * jnp.tanh(hz)
        o_ref[...] = x_ref[pl.ds(row0, T), :].astype(f32) + y * g

    @pl.when(i == 0)
    def _():
        for n, _, _ in pairs:
            copies[n].start()
        wait('vec0', 'vec1', 'vec2', 'vec3')
        init()
        wait('x0')
        a_ln(0, alt)
        wait('w1', 'x0b')
        a_ln(1, main)
        a_h1(alt, None, None)
        a_h1(main, alt, None)
        wait('bre')
        ur0 = _dot_nt(alt['xn2'][0:T, :], bre_ref[...])
        ur1 = _dot_nt(main['xn2'][0:T, :], bre_ref[...])
        wait('bim', 'cre', 'cim')
        ui0 = _dot_nt(alt['xn2'][0:T, :], bim_ref[...])
        a_store_u(alt, ur0, ui0)
        a_scan(alt)
        ui1 = _dot_nt(main['xn2'][0:T, :], bim_ref[...])
        a_store_u(main, ur1, ui1)
        a_scan(main)
        x1, y = stage_b_early(alt, True)
        stage_b_late(x1, y, True, pin=True)
        wait('x1')

    @pl.when(jnp.logical_and(i > 0, i < nsteps - 1))
    def _():
        x1, y = stage_b_early(main)
        stage_a(i + 1, i == nsteps - 2)
        a_ln(jnp.minimum(i + 2, nsteps - 1), main)
        stage_b_late(x1, y, pin=True)

    @pl.when(i == nsteps - 1)
    def _():
        x1, y = stage_b_early(main, c_late=True)
        stage_b_late(x1, y)


@jax.jit
def pallas_recurrent_scan__ssm_conv_s5__mixer_s_mlp__prompt_kernel(
    A_x, A_Lambda_re, A_Lambda_im, A_B_re, A_B_im, A_C_re, A_C_im, A_log_dt,
    A_Dskip, B_x, B_w1, B_w2, B_w3, B_w4,
):
    Bsz, L, D = A_x.shape
    P = A_Lambda_re.shape[0]
    F = B_w3.shape[1]
    T = _T
    nb = L // T
    assert Bsz == 1 and D == 640 and P == 640 and L % T == 0 and nb >= 3
    x2 = A_x.reshape(L, D)
    anyspec = pl.BlockSpec(memory_space=pl.ANY)
    bf16 = jnp.bfloat16
    blockbufs = [
        pltpu.VMEM((P // 128, _TP, 128), jnp.float32),
        pltpu.VMEM((P // 128, _TP, 128), jnp.float32),
        pltpu.VMEM((T + 8 + _HALO, D), jnp.float32),
        pltpu.VMEM((T, D), bf16),
        pltpu.VMEM((T + _HALO, D), bf16),
        pltpu.VMEM((T + _HALO, D), bf16),
        pltpu.VMEM((2, T, P), bf16),
    ]
    out = pl.pallas_call(
        functools.partial(_kernel, L=L, D=D),
        grid=(nb,),
        in_specs=[anyspec] * 13,
        out_specs=pl.BlockSpec((T, D), lambda i: (i, 0)),
        out_shape=jax.ShapeDtypeStruct((L, D), jnp.float32),
        scratch_shapes=[
            pltpu.VMEM((L, D), bf16),
            pltpu.VMEM((P,), bf16), pltpu.VMEM((P,), bf16),
            pltpu.VMEM((P,), bf16), pltpu.VMEM((D,), bf16),
            pltpu.VMEM((P, D), bf16), pltpu.VMEM((P, D), bf16),
            pltpu.VMEM((D, P), bf16), pltpu.VMEM((D, P), bf16),
            pltpu.VMEM((D, D), bf16), pltpu.VMEM((D, D), bf16),
            pltpu.VMEM((D, F), bf16), pltpu.VMEM((F, D), bf16),
            pltpu.SemaphoreType.DMA((16,)),
            pltpu.VMEM((16, P), jnp.float32),
            pltpu.VMEM((2, 8, P), jnp.float32),
        ] + blockbufs + blockbufs,
        compiler_params=pltpu.CompilerParams(
            dimension_semantics=("arbitrary",),
            vmem_limit_bytes=100 * 1024 * 1024,
        ),
    )(x2, A_Lambda_re, A_Lambda_im, A_log_dt, A_Dskip,
      A_B_re, A_B_im, A_C_re, A_C_im, B_w1, B_w2, B_w3, B_w4)
    return out.reshape(Bsz, L, D)
```

```python
import functools

import jax
import jax.numpy as jnp
from jax import lax
import jax.experimental.pallas as pl
import jax.experimental.pallas.tpu as pltpu

_EPS = 1e-5
_T = 256
_NV = 2
_NC = 8 * _NV
_CS = _T // _NC + 1
_TP = _CS * _NC
_HALO = 16
_RC = 32
_X0 = 2 * _T + _HALO
_X1 = 3 * _T + _HALO


def _ln(x):
    m = jnp.mean(x, axis=-1, keepdims=True)
    xc = x - m
    v = jnp.mean(xc * xc, axis=-1, keepdims=True)
    return xc * lax.rsqrt(v + _EPS)


def _gelu(x):
    c = 0.7978845608028654
    hx = 0.5 * x
    return hx + hx * jnp.tanh(x * (c + (c * 0.044715) * (x * x)))


def _dot_nn(a, b):
    return jnp.dot(a, b, preferred_element_type=jnp.float32)


def _dot_nt(a, b):
    return lax.dot_general(a, b, (((1,), (1,)), ((), ())),
                           preferred_element_type=jnp.float32)


def _cmul(ar, ai, br, bi):
    return ar * br - ai * bi, ar * bi + ai * br


def _kernel(x_hbm, lre_hbm, lim_hbm, ldt_hbm, dsk_hbm,
            bre_hbm, bim_hbm, cre_hbm, cim_hbm, w1_hbm, w2_hbm, w3_hbm, w4_hbm,
            o_ref,
            x_ref, lre_ref, lim_ref, ldt_ref, dsk_ref,
            bre_ref, bim_ref, cre_ref, cim_ref, w1_ref, w2_ref, w3_ref, w4_ref,
            sems, par_ref, carry_ref, *bufs, L, D):
    T, CS, NV = _T, _CS, _NV
    NJ = D // 128
    i = pl.program_id(0)
    nsteps = pl.num_programs(0)
    f32 = jnp.float32
    bf16 = jnp.bfloat16
    keys = ('ure', 'uim', 'h1', 'xn', 'xn2', 'xnn', 'hb')
    main = dict(zip(keys, bufs[:len(keys)]))
    alt = dict(zip(keys, bufs[len(keys):]))

    pairs = [
        ('vec0', lre_hbm, lre_ref), ('vec1', lim_hbm, lim_ref),
        ('vec2', ldt_hbm, ldt_ref), ('vec3', dsk_hbm, dsk_ref),
        ('x0', x_hbm.at[0:_T + _HALO], x_ref.at[0:_T + _HALO]),
        ('w1', w1_hbm, w1_ref),
        ('x0b', x_hbm.at[_T + _HALO:_X0], x_ref.at[_T + _HALO:_X0]), ('bre', bre_hbm, bre_ref), ('bim', bim_hbm, bim_ref),
        ('w2', w2_hbm, w2_ref), ('cre', cre_hbm, cre_ref), ('cim', cim_hbm, cim_ref),
        ('xa', x_hbm.at[_X0:_X1], x_ref.at[_X0:_X1]),
        ('w3', w3_hbm, w3_ref), ('w4', w4_hbm, w4_ref),
        ('x1', x_hbm.at[_X1:L], x_ref.at[_X1:L]),
    ]
    copies = {n: pltpu.make_async_copy(h, v, sems.at[k])
              for k, (n, h, v) in enumerate(pairs)}

    def wait(*ns):
        for n in ns:
            copies[n].wait()

    def init():
        lre = lre_ref[...].reshape(1, D).astype(f32)
        lim = lim_ref[...].reshape(1, D).astype(f32)
        dt = jnp.exp(ldt_ref[...].reshape(1, D).astype(f32)).astype(bf16).astype(f32)
        mag = jnp.exp(dt * lre)
        ang = dt * lim
        ar = mag * jnp.cos(ang)
        ai = mag * jnp.sin(ang)
        den = lre * lre + lim * lim
        nr = ar - 1.0
        ni = ai
        cr = (nr * lre + ni * lim) / den
        ci = (ni * lre - nr * lim) / den
        par_ref[0:1, :] = ar
        par_ref[1:2, :] = ai
        par_ref[2:3, :] = cr
        par_ref[3:4, :] = ci
        pr, pi = ar, ai
        n = 1
        while 2 * n <= CS:
            pr, pi = _cmul(pr, pi, pr, pi)
            n *= 2
        while n < CS:
            pr, pi = _cmul(pr, pi, ar, ai)
            n += 1
        for k in range(3):
            par_ref[4 + 2 * k:5 + 2 * k, :] = pr
            par_ref[5 + 2 * k:6 + 2 * k, :] = pi
            pr, pi = _cmul(pr, pi, pr, pi)
        par_ref[12:13, :] = dsk_ref[...].reshape(1, D).astype(f32)
        carry_ref[...] = jnp.zeros(carry_ref.shape, f32)
        for b in (main, alt):
            for j in range(NJ):
                b['ure'][j, T:_TP, :] = jnp.zeros((_TP - T, 128), f32)
                b['uim'][j, T:_TP, :] = jnp.zeros((_TP - T, 128), f32)

    def a_ln(blk, b):
        if isinstance(blk, int):
            row0 = blk * T
            hrow0 = row0 + T
        else:
            row0 = pl.multiple_of(blk * T, T)
            hrow0 = pl.multiple_of(jnp.minimum(row0 + T, L - _HALO), _HALO)

        def ln_rows(r0, nrows, src0):
            x = x_ref[pl.ds(src0, nrows), :].astype(f32)
            xn = _ln(x).astype(bf16)
            b['xn2'][r0:r0 + nrows, :] = xn
            b['xnn'][r0:r0 + nrows, :] = _ln(xn.astype(f32)).astype(bf16)

        for c in range(0, T, _RC):
            ln_rows(c, _RC, row0 + c)
        ln_rows(T, _HALO, hrow0)

    def a_store_u(b, ur, ui):
        bur, bui = _cmul(par_ref[2:3, :], par_ref[3:4, :], ur, ui)
        for j in range(NJ):
            b['ure'][j, 0:T, :] = bur[:, 128 * j:128 * (j + 1)]
            b['uim'][j, 0:T, :] = bui[:, 128 * j:128 * (j + 1)]

    def a_h1(b, prev, halo_zero):
        h1 = _gelu(_dot_nn(b['xnn'][...], w1_ref[...]))
        h1_ref = b['h1']
        if prev is None:
            h1_ref[0:8, :] = jnp.zeros((8, D), f32)
        else:
            h1_ref[0:8, :] = prev['h1'][T:T + 8, :]
        h1_ref[8:8 + T, :] = h1[:T]
        if halo_zero is None:
            h1_ref[8 + T:8 + T + _HALO, :] = h1[T:]
        else:
            h1_ref[8 + T:8 + T + _HALO, :] = jnp.where(halo_zero, 0.0, h1[T:])
        b['xn'][...] = b['xn2'][0:T, :]

    def a_scan(b):
        ure_ref, uim_ref = b['ure'], b['uim']
        ar = jnp.broadcast_to(par_ref[0:1, :], (8, D))
        ai = jnp.broadcast_to(par_ref[1:2, :], (8, D))
        sub = lax.broadcasted_iota(jnp.int32, (8, D), 0)

        def ld(ref, v, s):
            return jnp.concatenate(
                [ref[j, pl.ds(8 * CS * v + s, 8, stride=CS), :] for j in range(NJ)],
                axis=1)

        def st(ref, v, s, val):
            for j in range(NJ):
                ref[j, pl.ds(8 * CS * v + s, 8, stride=CS), :] = (
                    val[:, 128 * j:128 * (j + 1)])

        er = [jnp.zeros((8, D), f32) for _ in range(NV)]
        ei = [jnp.zeros((8, D), f32) for _ in range(NV)]
        for s in range(CS):
            for v in range(NV):
                br = ld(ure_ref, v, s)
                bi = ld(uim_ref, v, s)
                er[v], ei[v] = (ar * er[v] - ai * ei[v] + br,
                                ar * ei[v] + ai * er[v] + bi)
        inr, ini = carry_ref[0], carry_ref[1]
        hr, hi = [], []
        for v in range(NV):
            zr = jnp.where(sub == 0, pltpu.roll(inr, 1, 0), pltpu.roll(er[v], 1, 0))
            zi = jnp.where(sub == 0, pltpu.roll(ini, 1, 0), pltpu.roll(ei[v], 1, 0))
            for k in range(3):
                sh = 1 << k
                pr = par_ref[4 + 2 * k:5 + 2 * k, :]
                pi = par_ref[5 + 2 * k:6 + 2 * k, :]
                sr = jnp.where(sub >= sh, pltpu.roll(zr, sh, 0), 0.0)
                si = jnp.where(sub >= sh, pltpu.roll(zi, sh, 0), 0.0)
                tr, ti = _cmul(pr, pi, sr, si)
                zr = zr + tr
                zi = zi + ti
            hr.append(zr)
            hi.append(zi)
            if v + 1 < NV:
                tr, ti = _cmul(par_ref[4:5, :], par_ref[5:6, :], zr, zi)
                inr = tr + er[v]
                ini = ti + ei[v]
        for s in range(CS):
            for v in range(NV):
                br = ld(ure_ref, v, s)
                bi = ld(uim_ref, v, s)
                hr[v], hi[v] = (ar * hr[v] - ai * hi[v] + br,
                                ar * hi[v] + ai * hr[v] + bi)
                st(ure_ref, v, s, hr[v])
                st(uim_ref, v, s, hi[v])
        carry_ref[0] = jnp.concatenate(
            [ure_ref[j, T - 8:T, :] for j in range(NJ)], axis=1)
        carry_ref[1] = jnp.concatenate(
            [uim_ref[j, T - 8:T, :] for j in range(NJ)], axis=1)
        b['hb'][0] = jnp.concatenate([ure_ref[j, 0:T, :] for j in range(NJ)],
                                     axis=1).astype(bf16)
        b['hb'][1] = jnp.concatenate([uim_ref[j, 0:T, :] for j in range(NJ)],
                                     axis=1).astype(bf16)

    def stage_a(blk, halo_zero):
        xn_b = main['xn2'][0:T, :]
        ur = _dot_nt(xn_b, bre_ref[...])
        ui = _dot_nt(xn_b, bim_ref[...])
        a_store_u(main, ur, ui)
        a_h1(main, main, halo_zero)
        a_scan(main)

    def stage_b_early(b, first=False, c_late=False):
        lane = lax.broadcasted_iota(jnp.int32, (T, 128), 1)
        h1_ref = b['h1']
        xn = b['xn'][...].astype(f32)
        if not c_late:
            y = _dot_nt(b['hb'][0], cre_ref[...]) - _dot_nt(b['hb'][1], cim_ref[...])
            y = 2.0 * y + xn * par_ref[12:13, :]
        o = 8
        s0 = h1_ref[o - 1:o - 1 + T, 0:128]
        s1 = jnp.where(lane < 32, h1_ref[o - 1:o - 1 + T, 128:256],
                       h1_ref[o + 1:o + 1 + T, 128:256])
        s2 = jnp.where(lane < 64, h1_ref[o + 1:o + 1 + T, 256:384],
                       h1_ref[o - 2:o - 2 + T, 256:384])
        s3 = jnp.where(lane < 96, h1_ref[o - 2:o - 2 + T, 384:512],
                       h1_ref[o + 2:o + 2 + T, 384:512])
        s4 = h1_ref[o + 2:o + 2 + T, 512:640]
        sh_all = jnp.concatenate([s0, s1, s2, s3, s4], axis=1).astype(bf16)
        x1 = xn + _dot_nn(sh_all, w2_ref[...])
        if first:
            wait('cre', 'cim')
        if c_late:
            never = i < 0
            h0 = jnp.where(never, x1.astype(bf16), b['hb'][0])
            y = _dot_nt(h0, cre_ref[...]) - _dot_nt(b['hb'][1], cim_ref[...])
            y = 2.0 * y + xn * par_ref[12:13, :]
        return x1, y

    def stage_b_late(x1, y, first=False, pin=False):
        row0 = pl.multiple_of(i * T, T)
        x1n = _ln(x1).astype(bf16)
        if first:
            wait('xa', 'w3')
            a_ln(2, main)
        if not pin:
            h2 = _gelu(_dot_nn(x1n, w3_ref[...])).astype(bf16)
        else:
            never = i < 0
            nt = w3_ref.shape[1] // 128
            parts = []
            for t in range(nt):
                p = _gelu(_dot_nn(x1n, w3_ref[:, 128 * t:128 * (t + 1)]))
                c = t - 2
                if 0 <= c <= T // _RC:
                    r0 = c * _RC
                    nr = _RC if c < T // _RC else _HALO
                    ja = main['xnn'][r0:r0 + nr, :].astype(f32)
                    jb = main['xn2'][r0:r0 + nr, :].astype(f32)
                    junk = jnp.concatenate(
                        [ja[:, 128 * j:128 * (j + 1)] + jb[:, 128 * j:128 * (j + 1)]
                         for j in range(NJ)] + [p[NJ * nr:]], axis=0)
                    p = jnp.where(never, junk, p)
                parts.append(p.astype(bf16))
            h2 = jnp.concatenate(parts, axis=1)
        if first:
            wait('w4')
        z = x1 + _dot_nn(h2, w4_ref[...])
        hz = 0.5 * z
        g = hz + hz * jnp.tanh(hz)
        o_ref[...] = x_ref[pl.ds(row0, T), :].astype(f32) + y * g

    @pl.when(i == 0)
    def _():
        for n, _, _ in pairs:
            copies[n].start()
        wait('vec0', 'vec1', 'vec2', 'vec3')
        init()
        wait('x0')
        a_ln(0, alt)
        wait('w1', 'x0b')
        a_ln(1, main)
        a_h1(alt, None, None)
        a_h1(main, alt, None)
        wait('bre')
        ur0 = _dot_nt(alt['xn2'][0:T, :], bre_ref[...])
        ur1 = _dot_nt(main['xn2'][0:T, :], bre_ref[...])
        wait('bim', 'w2')
        ui0 = _dot_nt(alt['xn2'][0:T, :], bim_ref[...])
        a_store_u(alt, ur0, ui0)
        a_scan(alt)
        ui1 = _dot_nt(main['xn2'][0:T, :], bim_ref[...])
        a_store_u(main, ur1, ui1)
        a_scan(main)
        x1, y = stage_b_early(alt, True, c_late=True)
        stage_b_late(x1, y, True, pin=True)
        wait('x1')

    @pl.when(jnp.logical_and(i > 0, i < nsteps - 1))
    def _():
        x1, y = stage_b_early(main, c_late=True)
        stage_a(i + 1, i == nsteps - 2)
        a_ln(jnp.minimum(i + 2, nsteps - 1), main)
        stage_b_late(x1, y, pin=True)

    @pl.when(i == nsteps - 1)
    def _():
        x1, y = stage_b_early(main, c_late=True)
        stage_b_late(x1, y)


@jax.jit
def pallas_recurrent_scan__ssm_conv_s5__mixer_s_mlp__prompt_kernel(
    A_x, A_Lambda_re, A_Lambda_im, A_B_re, A_B_im, A_C_re, A_C_im, A_log_dt,
    A_Dskip, B_x, B_w1, B_w2, B_w3, B_w4,
):
    Bsz, L, D = A_x.shape
    P = A_Lambda_re.shape[0]
    F = B_w3.shape[1]
    T = _T
    nb = L // T
    assert Bsz == 1 and D == 640 and P == 640 and L % T == 0 and nb >= 4
    x2 = A_x.reshape(L, D)
    anyspec = pl.BlockSpec(memory_space=pl.ANY)
    bf16 = jnp.bfloat16
    blockbufs = [
        pltpu.VMEM((P // 128, _TP, 128), jnp.float32),
        pltpu.VMEM((P // 128, _TP, 128), jnp.float32),
        pltpu.VMEM((T + 8 + _HALO, D), jnp.float32),
        pltpu.VMEM((T, D), bf16),
        pltpu.VMEM((T + _HALO, D), bf16),
        pltpu.VMEM((T + _HALO, D), bf16),
        pltpu.VMEM((2, T, P), bf16),
    ]
    out = pl.pallas_call(
        functools.partial(_kernel, L=L, D=D),
        grid=(nb,),
        in_specs=[anyspec] * 13,
        out_specs=pl.BlockSpec((T, D), lambda i: (i, 0)),
        out_shape=jax.ShapeDtypeStruct((L, D), jnp.float32),
        scratch_shapes=[
            pltpu.VMEM((L, D), bf16),
            pltpu.VMEM((P,), bf16), pltpu.VMEM((P,), bf16),
            pltpu.VMEM((P,), bf16), pltpu.VMEM((D,), bf16),
            pltpu.VMEM((P, D), bf16), pltpu.VMEM((P, D), bf16),
            pltpu.VMEM((D, P), bf16), pltpu.VMEM((D, P), bf16),
            pltpu.VMEM((D, D), bf16), pltpu.VMEM((D, D), bf16),
            pltpu.VMEM((D, F), bf16), pltpu.VMEM((F, D), bf16),
            pltpu.SemaphoreType.DMA((16,)),
            pltpu.VMEM((16, P), jnp.float32),
            pltpu.VMEM((2, 8, P), jnp.float32),
        ] + blockbufs + blockbufs,
        compiler_params=pltpu.CompilerParams(
            dimension_semantics=("arbitrary",),
            vmem_limit_bytes=100 * 1024 * 1024,
        ),
    )(x2, A_Lambda_re, A_Lambda_im, A_log_dt, A_Dskip,
      A_B_re, A_B_im, A_C_re, A_C_im, B_w1, B_w2, B_w3, B_w4)
    return out.reshape(Bsz, L, D)
```
